```python
import os as _os
_os.environ.setdefault("JAX_PLATFORMS", "cpu")
import jax
import jax.numpy as jnp

def _softmax(x, axis=-1):
    return jax.nn.softmax(x, axis=axis)
def _gelu(x):
    return jax.nn.gelu(x, approximate=True)
def _silu(x):
    return jax.nn.silu(x)
def _sigmoid(x):
    return jax.nn.sigmoid(x)
def _layernorm(x, axis=-1, eps=1e-5):
    m = jnp.mean(x, axis=axis, keepdims=True)
    v = jnp.var(x, axis=axis, keepdims=True)
    return (x - m) / jnp.sqrt(v + eps)
def _scatter_add(tgt, idx, src, axis=0):
    return tgt.at[idx].add(src)
def _segment_sum(src, seg, n):
    return jax.ops.segment_sum(src, seg, n)
class _Rng:
    def __init__(self, key):
        self._k = key
    def _next(self):
        self._k, sub = jax.random.split(self._k)
        return sub
    def normal(self, shape):
        return jax.random.normal(self._next(), shape, dtype=jnp.bfloat16)
    def randint(self, lo, hi, shape):
        return jax.random.randint(self._next(), shape, lo, hi, dtype=jnp.int32)
    def uniform(self, shape, lo=0.0, hi=1.0):
        return jax.random.uniform(self._next(), shape, jnp.bfloat16, lo, hi)
    def permutation(self, n):
        return jax.random.permutation(self._next(), n)


kernel_name = 'standalone__gqa_block_cached__near_ridge'

def setup_inputs():
    _rng = _Rng(jax.random.key(int.from_bytes(__import__("os").urandom(4), "little")))
    _w = (lambda a: (lambda t: t.astype(jnp.bfloat16) if jnp.issubdtype(t.dtype, jnp.floating) else t)(jnp.asarray(a)))
    B, Sq, D = 8, 96, 448
    Hq, Hkv, Sk, Dh = 16, 8, 2048, 256
    assert Hq % Hkv == 0, (Hq, Hkv)
    return {
        "x": _w((lambda *s: _rng.normal(s) * 0.8)(B, Sq, D)),
        "k_cache": _w((lambda *s: _rng.normal(s) * 0.8)(B, Hkv, Sk, Dh)),
        "v_cache": _w((lambda *s: _rng.normal(s) * 0.05)(B, Hkv, Sk, Dh)),
        "wq": _w((lambda *s: _rng.normal(s) * 0.8)(D, Hq * Dh) * (D ** -0.5)),
        "wo": _w((lambda *s: _rng.normal(s) * 0.05)(Hq * Dh, D) * ((Hq * Dh) ** -0.5)),
    }

def reference(x, k_cache, v_cache, wq, wo):
    B, Sq, D = x.shape
    Hq, Dh = 16, 256
    Hkv = k_cache.shape[1]
    rep = Hq // Hkv
    q = (lambda x, *d: x.transpose(*d))((x @ wq).reshape(B, Sq, Hq, Dh), 0, 2, 1, 3)
    k = jnp.repeat(k_cache, rep, axis=1)
    v = jnp.repeat(v_cache, rep, axis=1)
    scores = jnp.einsum("bhqd,bhkd->bhqk", q, k) * (Dh ** -0.5)
    p = _softmax(scores, axis=-1)
    o = jnp.einsum("bhqk,bhkd->bhqd", p, v)
    return (lambda x, *d: x.transpose(*d))(o, 0, 2, 1, 3).reshape(B, Sq, Hq * Dh) @ wo
```

```python
import functools
import math
import jax
import jax.numpy as jnp
from jax import lax
import jax.experimental.pallas as pl
import jax.experimental.pallas.tpu as pltpu

HQ = 16
NSLOT = 4
_NT = (((1,), (1,)), ((), ()))


def _kernel(x_hbm, k_hbm, v_hbm, wq_hbm, wot_hbm, o_hbm,
            x_v, wq_v, wot_v, kbuf, vbuf, q_scr, o_scr, acc, out_v,
            sem_x, sem_wq, sem_wo, sem_k, sem_v, sem_o,
            *, B, Hkv, rep, sq, dh, qscale):
    nsteps = B * Hkv
    gw = rep * dh
    lb = B.bit_length() - 1
    assert B == 1 << lb and NSLOT & (NSLOT - 1) == 0

    def bh(n):
        if isinstance(n, int):
            return n % B, n // B
        return n & (B - 1), lax.shift_right_logical(n, lb)

    def k_copy(n):
        b, h = bh(n)
        slot = n & (NSLOT - 1)
        return pltpu.make_async_copy(k_hbm.at[b, h], kbuf.at[slot], sem_k.at[slot])

    def v_copy(n):
        b, h = bh(n)
        slot = n & (NSLOT - 1)
        return pltpu.make_async_copy(v_hbm.at[b, h], vbuf.at[slot], sem_v.at[slot])

    def wq_copy(h):
        return pltpu.make_async_copy(wq_hbm.at[:, pl.ds(pl.multiple_of(h * gw, gw), gw)], wq_v.at[h], sem_wq.at[h])

    def wo_copy(h):
        return pltpu.make_async_copy(wot_hbm.at[:, pl.ds(pl.multiple_of(h * gw, gw), gw)], wot_v.at[h], sem_wo.at[h])

    def out_copy(b):
        return pltpu.make_async_copy(out_v.at[b], o_hbm.at[b], sem_o.at[b])

    x0_copy = pltpu.make_async_copy(x_hbm.at[pl.ds(0, 1)], x_v.at[pl.ds(0, 1)], sem_x.at[0])
    xr_copy = pltpu.make_async_copy(x_hbm.at[pl.ds(1, B - 1)], x_v.at[pl.ds(1, B - 1)], sem_x.at[1])

    def q_proj(n):
        b, h = bh(n)
        qn = jnp.dot(x_v[b], wq_v[h], preferred_element_type=jnp.float32) * qscale
        qn = qn.astype(jnp.bfloat16)
        for r in range(rep):
            q_scr[r * sq:(r + 1) * sq, :] = qn[:, r * dh:(r + 1) * dh]

    def o_proj(n):
        b, h = bh(n)
        y = lax.dot_general(o_scr[...], wot_v[h], _NT, preferred_element_type=jnp.float32)
        acc[b] = y + jnp.where(h > 0, acc[b], 0.0)

    x0_copy.start()
    wq_copy(0).start()
    k_copy(0).start()
    xr_copy.start()
    v_copy(0).start()
    wo_copy(0).start()
    for s in range(1, NSLOT):
        k_copy(s).start()
        v_copy(s).start()
    o_scr[...] = jnp.zeros(o_scr.shape, o_scr.dtype)
    x0_copy.wait()
    wq_copy(0).wait()
    q_proj(0)
    xr_copy.wait()
    wo_copy(0).wait()

    def body(n, carry):
        b, h = bh(n)
        slot = n & (NSLOT - 1)

        @pl.when(jnp.logical_and(b == B - 1, h + 1 < Hkv))
        def _():
            wq_copy(h + 1).wait()

        @pl.when(jnp.logical_and(b == 1, h > 0))
        def _():
            wo_copy(h).wait()

        k_copy(n).wait()
        v_copy(n).wait()

        n_prev = jnp.maximum(n - 1, 0)
        q2 = q_scr[...]
        s = lax.dot_general(q2, kbuf[slot], _NT, preferred_element_type=jnp.float32)
        o_proj(n_prev)
        m = jnp.max(s, axis=-1, keepdims=True)
        p = jnp.exp2(s - m)
        l = jnp.sum(p, axis=-1, keepdims=True)
        o = jnp.dot(p.astype(jnp.bfloat16), vbuf[slot], preferred_element_type=jnp.float32)
        q_proj(jnp.minimum(n + 1, nsteps - 1))
        o = (o / l).astype(jnp.bfloat16)
        for r in range(rep):
            o_scr[:, r * dh:(r + 1) * dh] = o[r * sq:(r + 1) * sq, :]

        @pl.when(n + NSLOT < nsteps)
        def _():
            k_copy(n + NSLOT).start()
            v_copy(n + NSLOT).start()

        @pl.when(jnp.logical_and(b == 2, h + 1 < Hkv))
        def _():
            wq_copy(h + 1).start()

        @pl.when(jnp.logical_and(b == 4, h + 1 < Hkv))
        def _():
            wo_copy(h + 1).start()

        @pl.when(n_prev >= nsteps - B)
        def _():
            bp = n_prev & (B - 1)
            out_v[bp] = acc[bp].astype(out_v.dtype)
            out_copy(bp).start()

        return carry

    lax.fori_loop(0, nsteps, body, 0)

    o_proj(nsteps - 1)
    out_v[B - 1] = acc[B - 1].astype(out_v.dtype)
    out_copy(B - 1).start()
    for b in range(B):
        out_copy(b).wait()


@jax.jit
def pallas_standalone__gqa_block_cached__near_ridge_kernel(x, k_cache, v_cache, wq, wo):
    B, Sq, D = x.shape
    _, Hkv, Sk, Dh = k_cache.shape
    rep = HQ // Hkv
    gw = rep * Dh
    kern = functools.partial(_kernel, B=B, Hkv=Hkv, rep=rep, sq=Sq, dh=Dh,
                             qscale=(Dh ** -0.5) * math.log2(math.e))
    bf = jnp.bfloat16
    return pl.pallas_call(
        kern,
        in_specs=[pl.BlockSpec(memory_space=pl.ANY)] * 5,
        out_specs=pl.BlockSpec(memory_space=pl.ANY),
        out_shape=jax.ShapeDtypeStruct((B, Sq, D), x.dtype),
        scratch_shapes=[
            pltpu.VMEM((B, Sq, D), bf),
            pltpu.VMEM((Hkv, D, gw), bf),
            pltpu.VMEM((Hkv, D, gw), bf),
            pltpu.VMEM((NSLOT, Sk, Dh), bf),
            pltpu.VMEM((NSLOT, Sk, Dh), bf),
            pltpu.VMEM((rep * Sq, Dh), bf),
            pltpu.VMEM((Sq, gw), bf),
            pltpu.VMEM((B, Sq, D), jnp.float32),
            pltpu.VMEM((B, Sq, D), bf),
            pltpu.SemaphoreType.DMA((2,)),
            pltpu.SemaphoreType.DMA((Hkv,)),
            pltpu.SemaphoreType.DMA((Hkv,)),
            pltpu.SemaphoreType.DMA((NSLOT,)),
            pltpu.SemaphoreType.DMA((NSLOT,)),
            pltpu.SemaphoreType.DMA((B,)),
        ],
        compiler_params=pltpu.CompilerParams(vmem_limit_bytes=64 * 1024 * 1024,
                                             disable_bounds_checks=True),
    )(x, k_cache, v_cache, wq, wo.T)
```

```python
import functools
import math

import jax
import jax.numpy as jnp
from jax import lax
import jax.experimental.pallas as pl
import jax.experimental.pallas.tpu as pltpu

_HQ = 16
_NSLOT = 2
_WQ_AT = 1
_WO_AT = 5
_LANES = 128
_NT = (((1,), (1,)), ((), ()))


def _kernel(x_hbm, k_hbm, v_hbm, wq_hbm, wot_hbm, o_hbm,
            x_v, wq_v, wot_v, kbuf, vbuf, q_all, o_scr, acc, out_v,
            sem_x, sem_wq, sem_wo, sem_k, sem_v, sem_o,
            *, nb, nh, rep, sq, dh, qscale):
    nsteps = nb * nh
    gw = rep * dh
    log_nb = nb.bit_length() - 1
    f32, bf16 = jnp.float32, jnp.bfloat16

    def bh(n):
        if isinstance(n, int):
            return n % nb, n // nb
        return n & (nb - 1), lax.shift_right_logical(n, log_nb)

    def k_copy(n):
        b, h = bh(n)
        slot = n & (_NSLOT - 1)
        return pltpu.make_async_copy(k_hbm.at[b, h], kbuf.at[slot], sem_k.at[slot])

    def v_copy(n):
        b, h = bh(n)
        slot = n & (_NSLOT - 1)
        return pltpu.make_async_copy(v_hbm.at[b, h], vbuf.at[slot], sem_v.at[slot])

    def w_slice(w_hbm, h):
        return w_hbm.at[:, pl.ds(pl.multiple_of(h * gw, gw), gw)]

    def wq_copy(h):
        return pltpu.make_async_copy(w_slice(wq_hbm, h), wq_v.at[h], sem_wq.at[h])

    def wo_copy(h):
        return pltpu.make_async_copy(w_slice(wot_hbm, h), wot_v.at[h], sem_wo.at[h])

    x_copy = pltpu.make_async_copy(x_hbm, x_v, sem_x.at[0])
    out_head_copy = pltpu.make_async_copy(
        out_v.at[pl.ds(0, nb - 1)], o_hbm.at[pl.ds(0, nb - 1)], sem_o.at[0])
    out_tail_copy = pltpu.make_async_copy(
        out_v.at[pl.ds(nb - 1, 1)], o_hbm.at[pl.ds(nb - 1, 1)], sem_o.at[1])

    def q_proj(b, h):
        q = jnp.dot(x_v[b], wq_v[h], preferred_element_type=f32) * qscale
        q = q.astype(bf16)
        for r in range(rep):
            q_all[b, r * sq:(r + 1) * sq, :] = q[:, r * dh:(r + 1) * dh]

    def o_proj(n):
        b, h = bh(n)
        y = lax.dot_general(o_scr[...], wot_v[h], _NT, preferred_element_type=f32)
        acc[b] = y + jnp.where(h > 0, acc[b], 0.0)

    x_copy.start()
    wq_copy(0).start()
    k_copy(0).start()
    wo_copy(0).start()
    v_copy(0).start()
    wq_copy(1).start()
    k_copy(1).start()
    o_scr[...] = jnp.zeros(o_scr.shape, o_scr.dtype)
    x_copy.wait()
    wq_copy(0).wait()
    for b in range(nb):
        q_proj(b, 0)
    wo_copy(0).wait()

    def main_body(n, carry):
        b, h = bh(n)
        slot = n & (_NSLOT - 1)

        @pl.when(jnp.logical_and(b == 1, h > 0))
        def _():
            wo_copy(h).wait()

        k_copy(n).wait()
        v_copy(n + 1).start()

        @pl.when(jnp.logical_and(b == _WQ_AT, h + 2 < nh))
        def _():
            wq_copy(h + 2).start()

        @pl.when(b == _WO_AT)
        def _():
            wo_copy(h + 1).start()

        s = lax.dot_general(q_all[b], kbuf[slot], _NT, preferred_element_type=f32)
        o_proj(jnp.maximum(n - 1, 0))
        m = jnp.max(s, axis=-1, keepdims=True)

        @pl.when(b == 0)
        def _():
            wq_copy(h + 1).wait()

        v_copy(n).wait()
        k_copy(n + 2).start()

        q_proj(b, h + 1)
        p = jnp.exp2(s - m)
        l = jnp.sum(p, axis=-1, keepdims=True)
        o = jnp.dot(p.astype(bf16), vbuf[slot], preferred_element_type=f32)
        o = (o / l).astype(bf16)
        for r in range(rep):
            o_scr[:, r * dh:(r + 1) * dh] = o[r * sq:(r + 1) * sq, :]
        return carry

    def last_body(n, carry):
        b = n & (nb - 1)
        h = nh - 1
        slot = n & (_NSLOT - 1)

        k_copy(n).wait()

        @pl.when(n + 1 < nsteps)
        def _():
            v_copy(n + 1).start()

        s = lax.dot_general(q_all[b], kbuf[slot], _NT, preferred_element_type=f32)
        m = jnp.max(s, axis=-1, keepdims=True)

        @pl.when(b == nb - 1)
        def _():
            v_copy(n).wait()
            out_head_copy.start()

        @pl.when(b < nb - 1)
        def _():
            v_copy(n).wait()

        @pl.when(n + 2 < nsteps)
        def _():
            k_copy(n + 2).start()

        p = jnp.exp2(s - m)
        l = jnp.sum(p, axis=-1, keepdims=True)
        p = p.astype(bf16)
        y = acc[b]
        chunks = []
        for c in range(dh // _LANES):
            oc = jnp.dot(p, vbuf[slot, :, c * _LANES:(c + 1) * _LANES],
                         preferred_element_type=f32)
            chunks.append((oc / l).astype(bf16))
        for c, oc in enumerate(chunks):
            for r in range(rep):
                col = r * dh + c * _LANES
                y = y + lax.dot_general(oc[r * sq:(r + 1) * sq, :],
                                        wot_v[h, :, col:col + _LANES], _NT,
                                        preferred_element_type=f32)
        out_v[b] = y.astype(out_v.dtype)
        return carry

    lax.fori_loop(0, nsteps - nb, main_body, 0)
    o_proj(nsteps - nb - 1)
    wo_copy(nh - 1).wait()
    lax.fori_loop(nsteps - nb, nsteps, last_body, 0)

    out_tail_copy.start()
    out_head_copy.wait()
    out_tail_copy.wait()


@jax.jit
def pallas_standalone__gqa_block_cached__near_ridge_kernel(
    x: jax.Array,
    k_cache: jax.Array,
    v_cache: jax.Array,
    wq: jax.Array,
    wo: jax.Array,
):
    nb, sq, d = x.shape
    _, nh, sk, dh = k_cache.shape
    rep = _HQ // nh
    gw = rep * dh
    assert nb & (nb - 1) == 0 and nb > max(_WQ_AT, _WO_AT) and nh >= 2
    assert dh % _LANES == 0
    kern = functools.partial(
        _kernel, nb=nb, nh=nh, rep=rep, sq=sq, dh=dh,
        qscale=(dh ** -0.5) * math.log2(math.e))
    bf16 = jnp.bfloat16
    return pl.pallas_call(
        kern,
        in_specs=[pl.BlockSpec(memory_space=pl.ANY)] * 5,
        out_specs=pl.BlockSpec(memory_space=pl.ANY),
        out_shape=jax.ShapeDtypeStruct((nb, sq, d), x.dtype),
        scratch_shapes=[
            pltpu.VMEM((nb, sq, d), bf16),
            pltpu.VMEM((nh, d, gw), bf16),
            pltpu.VMEM((nh, d, gw), bf16),
            pltpu.VMEM((_NSLOT, sk, dh), bf16),
            pltpu.VMEM((_NSLOT, sk, dh), bf16),
            pltpu.VMEM((nb, rep * sq, dh), bf16),
            pltpu.VMEM((sq, gw), bf16),
            pltpu.VMEM((nb, sq, d), jnp.float32),
            pltpu.VMEM((nb, sq, d), bf16),
            pltpu.SemaphoreType.DMA((1,)),
            pltpu.SemaphoreType.DMA((nh,)),
            pltpu.SemaphoreType.DMA((nh,)),
            pltpu.SemaphoreType.DMA((_NSLOT,)),
            pltpu.SemaphoreType.DMA((_NSLOT,)),
            pltpu.SemaphoreType.DMA((2,)),
        ],
        compiler_params=pltpu.CompilerParams(
            vmem_limit_bytes=64 * 1024 * 1024,
            disable_bounds_checks=True,
        ),
    )(x, k_cache, v_cache, wq, wo.T)
```

```python
import functools
import math

import jax
import jax.numpy as jnp
from jax import lax
import jax.experimental.pallas as pl
import jax.experimental.pallas.tpu as pltpu

_HQ = 16
_NSLOT = 4
_WQ_AT = 1
_WO_AT = 5
_LANES = 128
_NT = (((1,), (1,)), ((), ()))


class _Split:
    def __init__(self, src, dst, sems, first_sem):
        self._args = (src, dst, sems, first_sem)

    def _part(self, i):
        src, dst, sems, first_sem = self._args
        half = src.shape[0] // 2
        return pltpu.make_async_copy(src.at[pl.ds(i * half, half)],
                                     dst.at[pl.ds(i * half, half)],
                                     sems.at[first_sem + i])

    def start_lo(self, priority=1):
        self._part(0).start(priority=priority)

    def start_hi(self):
        self._part(1).start(priority=0)

    def start(self, lo_priority):
        self.start_hi()
        self.start_lo(lo_priority)

    def wait(self):
        self._part(0).wait()
        self._part(1).wait()


def _kernel(x_hbm, k_hbm, v_hbm, wq_hbm, wot_hbm, o_hbm,
            x_v, wq_v, wot_v, kbuf, vbuf, q_all, o_scr, acc, out_v,
            sem_x, sem_wq, sem_wo, sem_k, sem_v, sem_o, sem_fence,
            *, nb, nh, rep, sq, dh, qscale):
    nsteps = nb * nh
    gw = rep * dh
    log_nb = nb.bit_length() - 1
    f32, bf16 = jnp.float32, jnp.bfloat16

    def bh(n):
        if isinstance(n, int):
            return n % nb, n // nb
        return n & (nb - 1), lax.shift_right_logical(n, log_nb)

    def k_copy(n):
        b, h = bh(n)
        slot = n & (_NSLOT - 1)
        return _Split(k_hbm.at[b, h], kbuf.at[slot], sem_k, 2 * slot)

    def v_copy(n):
        b, h = bh(n)
        slot = n & (_NSLOT - 1)
        return _Split(v_hbm.at[b, h], vbuf.at[slot], sem_v, 2 * slot)

    def w_slice(w_hbm, h):
        return w_hbm.at[:, pl.ds(pl.multiple_of(h * gw, gw), gw)]

    def wq_copy(h):
        return _Split(w_slice(wq_hbm, h), wq_v.at[h], sem_wq, 2 * h)

    def wo_copy(h):
        return _Split(w_slice(wot_hbm, h), wot_v.at[h], sem_wo, 2 * h)

    x_copy = _Split(x_hbm, x_v, sem_x, 0)
    out_head_copy = pltpu.make_async_copy(
        out_v.at[pl.ds(0, nb - 1)], o_hbm.at[pl.ds(0, nb - 1)], sem_o.at[0])
    out_tail_copy = pltpu.make_async_copy(
        out_v.at[pl.ds(nb - 1, 1)], o_hbm.at[pl.ds(nb - 1, 1)], sem_o.at[1])

    def q_proj(b, h):
        q = jnp.dot(x_v[b], wq_v[h], preferred_element_type=f32) * qscale
        q = q.astype(bf16)
        for r in range(rep):
            q_all[b, r * sq:(r + 1) * sq, :] = q[:, r * dh:(r + 1) * dh]

    def o_proj(n):
        b, h = bh(n)
        y = lax.dot_general(o_scr[...], wot_v[h], _NT, preferred_element_type=f32)
        acc[b] = y + jnp.where(h > 0, acc[b], 0.0)

    x_copy.start(0)
    wq_copy(0).start(0)
    k_copy(0).start(0)
    wo_copy(0).start(0)
    wq_copy(1).start(0)
    v_copy(0).start_lo()
    k_copy(1).start_lo()
    v_copy(1).start_lo()
    k_copy(2).start_lo()
    o_scr[...] = jnp.zeros(o_scr.shape, o_scr.dtype)
    x_copy.wait()
    wq_copy(0).wait()
    for b in range(nb):
        q_proj(b, 0)
    wo_copy(0).wait()


    def main_body(n, carry):
        b, h = bh(n)
        slot = n & (_NSLOT - 1)

        k_copy(n).wait()
        v_copy(n).start_hi()
        v_copy(n + 2).start_lo()

        @pl.when(jnp.logical_and(b == 1, h > 0))
        def _():
            wo_copy(h).wait()

        @pl.when(jnp.logical_and(b == _WQ_AT, h + 2 < nh))
        def _():
            wq_copy(h + 2).start(1)

        @pl.when(b == _WO_AT)
        def _():
            wo_copy(h + 1).start(1)

        s = lax.dot_general(q_all[b], kbuf[slot], _NT, preferred_element_type=f32)
        o_proj(jnp.maximum(n - 1, 0))
        m = jnp.max(s, axis=-1, keepdims=True)

        v_copy(n).wait()
        k_copy(n + 1).start_hi()
        k_copy(n + 3).start_lo()

        @pl.when(b == 0)
        def _():
            wq_copy(h + 1).wait()

        q_proj(b, h + 1)
        p = jnp.exp2(s - m)
        l = jnp.sum(p, axis=-1, keepdims=True)
        o = jnp.dot(p.astype(bf16), vbuf[slot], preferred_element_type=f32)
        o = (o / l).astype(bf16)
        for r in range(rep):
            o_scr[:, r * dh:(r + 1) * dh] = o[r * sq:(r + 1) * sq, :]
        return carry

    def last_body(n, carry):
        b = n & (nb - 1)
        h = nh - 1
        slot = n & (_NSLOT - 1)

        k_copy(n).wait()
        v_copy(n).start_hi()

        @pl.when(b < nb - 2)
        def _():
            v_copy(n + 2).start_lo()

        @pl.when(b == 0)
        def _():
            wo_copy(h).wait()

        s = lax.dot_general(q_all[b], kbuf[slot], _NT, preferred_element_type=f32)
        m = jnp.max(s, axis=-1, keepdims=True)

        @pl.when(b < nb - 1)
        def _():
            v_copy(n).wait()
            k_copy(n + 1).start_hi()

        @pl.when(b < nb - 3)
        def _():
            k_copy(n + 3).start_lo()

        @pl.when(b == nb - 1)
        def _():
            v_copy(n).wait()
            out_head_copy.start()

        pl.semaphore_signal(sem_fence, 1)
        pl.semaphore_wait(sem_fence, 1)

        p = jnp.exp2(s - m)
        l = jnp.sum(p, axis=-1, keepdims=True)
        p = p.astype(bf16)
        y = acc[b]
        chunks = []
        for c in range(dh // _LANES):
            oc = jnp.dot(p, vbuf[slot, :, c * _LANES:(c + 1) * _LANES],
                         preferred_element_type=f32)
            chunks.append((oc / l).astype(bf16))
        for c, oc in enumerate(chunks):
            for r in range(rep):
                col = r * dh + c * _LANES
                y = y + lax.dot_general(oc[r * sq:(r + 1) * sq, :],
                                        wot_v[h, :, col:col + _LANES], _NT,
                                        preferred_element_type=f32)
        out_v[b] = y.astype(out_v.dtype)
        return carry

    lax.fori_loop(0, nsteps - nb, main_body, 0)
    o_proj(nsteps - nb - 1)
    lax.fori_loop(nsteps - nb, nsteps, last_body, 0)

    out_tail_copy.start()
    out_head_copy.wait()
    out_tail_copy.wait()


@jax.jit
def pallas_standalone__gqa_block_cached__near_ridge_kernel(
    x: jax.Array,
    k_cache: jax.Array,
    v_cache: jax.Array,
    wq: jax.Array,
    wo: jax.Array,
):
    nb, sq, d = x.shape
    _, nh, sk, dh = k_cache.shape
    rep = _HQ // nh
    gw = rep * dh
    assert nb & (nb - 1) == 0 and nb > max(_WQ_AT, _WO_AT, 3) and nh >= 2
    assert dh % _LANES == 0 and sk % 32 == 0 and d % 32 == 0
    kern = functools.partial(
        _kernel, nb=nb, nh=nh, rep=rep, sq=sq, dh=dh,
        qscale=(dh ** -0.5) * math.log2(math.e))
    bf16 = jnp.bfloat16
    return pl.pallas_call(
        kern,
        in_specs=[pl.BlockSpec(memory_space=pl.ANY)] * 5,
        out_specs=pl.BlockSpec(memory_space=pl.ANY),
        out_shape=jax.ShapeDtypeStruct((nb, sq, d), x.dtype),
        scratch_shapes=[
            pltpu.VMEM((nb, sq, d), bf16),
            pltpu.VMEM((nh, d, gw), bf16),
            pltpu.VMEM((nh, d, gw), bf16),
            pltpu.VMEM((_NSLOT, sk, dh), bf16),
            pltpu.VMEM((_NSLOT, sk, dh), bf16),
            pltpu.VMEM((nb, rep * sq, dh), bf16),
            pltpu.VMEM((sq, gw), bf16),
            pltpu.VMEM((nb, sq, d), jnp.float32),
            pltpu.VMEM((nb, sq, d), bf16),
            pltpu.SemaphoreType.DMA((2,)),
            pltpu.SemaphoreType.DMA((2 * nh,)),
            pltpu.SemaphoreType.DMA((2 * nh,)),
            pltpu.SemaphoreType.DMA((2 * _NSLOT,)),
            pltpu.SemaphoreType.DMA((2 * _NSLOT,)),
            pltpu.SemaphoreType.DMA((2,)),
            pltpu.SemaphoreType.REGULAR,
        ],
        compiler_params=pltpu.CompilerParams(
            vmem_limit_bytes=64 * 1024 * 1024,
            disable_bounds_checks=True,
        ),
    )(x, k_cache, v_cache, wq, wo.T)
```

```python
import functools
import math

import jax
import jax.numpy as jnp
from jax import lax
import jax.experimental.pallas as pl
import jax.experimental.pallas.tpu as pltpu

_HQ = 16
_NSLOT = 4
_WQ_AT = 1
_WO_AT = 5
_NP = 16
_HI_FRAC = 8
_X_HEAD = 3
_LANES = 128
_NT = (((1,), (1,)), ((), ()))


class _Copy:
    def __init__(self, src, dst, sems, first_sem, hi=None):
        self._args = (src, dst, sems, first_sem)
        n = src.shape[0]
        self._hi = n // 2 if hi is None else hi
        self._lo = n - self._hi

    def _part(self, start, size, sem):
        src, dst, sems, first_sem = self._args
        return pltpu.make_async_copy(src.at[pl.ds(start, size)],
                                     dst.at[pl.ds(start, size)],
                                     sems.at[first_sem + sem])

    def start_lo(self, priority=1):
        self._part(0, self._lo, 0).start(priority=priority)

    def start_hi(self):
        self._part(self._lo, self._hi, 1).start(priority=0)

    def start_piece(self, j):
        size = self._hi // _NP
        self._part(self._lo + j * size, size, 1).start(priority=0)

    def start(self, lo_priority):
        self.start_hi()
        self.start_lo(lo_priority)

    def wait(self):
        self._part(0, self._lo, 0).wait()
        self._part(self._lo, self._hi, 1).wait()


def _kernel(x_hbm, k_hbm, v_hbm, wq_hbm, wot_hbm, o_hbm,
            x_v, wq_v, wot_v, kbuf, vbuf, q_all, o_scr, acc, out_v,
            sem_x, sem_wq, sem_wo, sem_k, sem_v, sem_o, sem_fence,
            *, nb, nh, rep, sq, sk, dh, qscale):
    nsteps = nb * nh
    gw = rep * dh
    ck = sk // _NP
    log_nb = nb.bit_length() - 1
    f32, bf16 = jnp.float32, jnp.bfloat16

    def bh(n):
        if isinstance(n, int):
            return n % nb, n // nb
        return n & (nb - 1), lax.shift_right_logical(n, log_nb)

    def k_copy(n):
        b, h = bh(n)
        slot = n & (_NSLOT - 1)
        return _Copy(k_hbm.at[b, h], kbuf.at[slot], sem_k, 2 * slot, sk // _HI_FRAC)

    def v_copy(n):
        b, h = bh(n)
        slot = n & (_NSLOT - 1)
        return _Copy(v_hbm.at[b, h], vbuf.at[slot], sem_v, 2 * slot, sk // _HI_FRAC)

    def w_slice(w_hbm, h):
        return w_hbm.at[:, pl.ds(pl.multiple_of(h * gw, gw), gw)]

    def wq_copy(h):
        return _Copy(w_slice(wq_hbm, h), wq_v.at[h], sem_wq, 2 * h)

    def wo_copy(h):
        return _Copy(w_slice(wot_hbm, h), wot_v.at[h], sem_wo, 2 * h)

    x_head_copy = pltpu.make_async_copy(
        x_hbm.at[pl.ds(0, _X_HEAD)], x_v.at[pl.ds(0, _X_HEAD)], sem_x.at[0])
    x_tail_copy = pltpu.make_async_copy(
        x_hbm.at[pl.ds(_X_HEAD, nb - _X_HEAD)], x_v.at[pl.ds(_X_HEAD, nb - _X_HEAD)],
        sem_x.at[1])
    out_head_copy = pltpu.make_async_copy(
        out_v.at[pl.ds(0, nb - 1)], o_hbm.at[pl.ds(0, nb - 1)], sem_o.at[0])
    out_tail_copy = pltpu.make_async_copy(
        out_v.at[pl.ds(nb - 1, 1)], o_hbm.at[pl.ds(nb - 1, 1)], sem_o.at[1])

    def q_proj(b, h):
        q = jnp.dot(x_v[b], wq_v[h], preferred_element_type=f32) * qscale
        q = q.astype(bf16)
        for r in range(rep):
            q_all[b, r * sq:(r + 1) * sq, :] = q[:, r * dh:(r + 1) * dh]

    def o_proj(n):
        b, h = bh(n)
        y = lax.dot_general(o_scr[...], wot_v[h], _NT, preferred_element_type=f32)
        acc[b] = y + jnp.where(h > 0, acc[b], 0.0)

    def scores(b, slot, issue):
        q = q_all[b]
        parts = []
        for c in range(_NP):
            parts.append(lax.dot_general(q, kbuf[slot, c * ck:(c + 1) * ck, :], _NT,
                                         preferred_element_type=f32))
            issue(c)
        return jnp.concatenate(parts, axis=1)

    def weighted_values(p, slot, issue):
        o = None
        for c in range(_NP):
            oc = jnp.dot(p[:, c * ck:(c + 1) * ck], vbuf[slot, c * ck:(c + 1) * ck, :],
                         preferred_element_type=f32)
            o = oc if o is None else o + oc
            issue(c)
        return o

    wq_copy(0).start(0)
    x_head_copy.start()
    x_tail_copy.start()
    k_copy(0).start(0)
    wo_copy(0).start(0)
    wq_copy(1).start(0)
    v_copy(0).start(1)
    k_copy(1).start_lo()
    v_copy(1).start_lo()
    k_copy(2).start_lo()
    o_scr[...] = jnp.zeros(o_scr.shape, o_scr.dtype)
    wq_copy(0).wait()
    x_head_copy.wait()
    for b in range(_X_HEAD):
        q_proj(b, 0)
    x_tail_copy.wait()
    for b in range(_X_HEAD, nb):
        q_proj(b, 0)
    wo_copy(0).wait()


    def main_body(n, carry):
        b, h = bh(n)
        slot = n & (_NSLOT - 1)

        k_copy(n).wait()
        v_copy(n + 2).start_lo()

        @pl.when(jnp.logical_and(b == 1, h > 0))
        def _():
            wo_copy(h).wait()

        @pl.when(jnp.logical_and(b == _WQ_AT, h + 2 < nh))
        def _():
            wq_copy(h + 2).start(1)

        @pl.when(b == _WO_AT)
        def _():
            wo_copy(h + 1).start(1)

        s = scores(b, slot, k_copy(n + 1).start_piece)
        o_proj(jnp.maximum(n - 1, 0))
        m = jnp.max(s, axis=-1, keepdims=True)

        v_copy(n).wait()
        k_copy(n + 3).start_lo()

        @pl.when(b == 0)
        def _():
            wq_copy(h + 1).wait()

        q_proj(b, h + 1)
        p = jnp.exp2(s - m)
        l = jnp.sum(p, axis=-1, keepdims=True)
        o = weighted_values(p.astype(bf16), slot, v_copy(n + 1).start_piece)
        o = (o / l).astype(bf16)
        for r in range(rep):
            o_scr[:, r * dh:(r + 1) * dh] = o[r * sq:(r + 1) * sq, :]
        return carry

    def last_body(n, carry):
        b = n & (nb - 1)
        h = nh - 1
        slot = n & (_NSLOT - 1)

        k_copy(n).wait()

        @pl.when(b < nb - 2)
        def _():
            v_copy(n + 2).start_lo()

        @pl.when(b == 0)
        def _():
            wo_copy(h).wait()

        def issue_k(c):
            @pl.when(b < nb - 1)
            def _():
                k_copy(n + 1).start_piece(c)

        s = scores(b, slot, issue_k)
        m = jnp.max(s, axis=-1, keepdims=True)

        @pl.when(b < nb - 1)
        def _():
            v_copy(n).wait()
            v_copy(n + 1).start_hi()

        @pl.when(b < nb - 3)
        def _():
            k_copy(n + 3).start_lo()

        @pl.when(b == nb - 1)
        def _():
            v_copy(n).wait()
            out_head_copy.start()

        pl.semaphore_signal(sem_fence, 1)
        pl.semaphore_wait(sem_fence, 1)

        p = jnp.exp2(s - m)
        l = jnp.sum(p, axis=-1, keepdims=True)
        p = p.astype(bf16)
        y = acc[b]
        chunks = []
        for c in range(dh // _LANES):
            oc = jnp.dot(p, vbuf[slot, :, c * _LANES:(c + 1) * _LANES],
                         preferred_element_type=f32)
            chunks.append((oc / l).astype(bf16))
        for c, oc in enumerate(chunks):
            for r in range(rep):
                col = r * dh + c * _LANES
                y = y + lax.dot_general(oc[r * sq:(r + 1) * sq, :],
                                        wot_v[h, :, col:col + _LANES], _NT,
                                        preferred_element_type=f32)
        out_v[b] = y.astype(out_v.dtype)
        return carry

    lax.fori_loop(0, nsteps - nb, main_body, 0)
    o_proj(nsteps - nb - 1)
    lax.fori_loop(nsteps - nb, nsteps, last_body, 0)

    out_tail_copy.start()
    out_head_copy.wait()
    out_tail_copy.wait()


@jax.jit
def pallas_standalone__gqa_block_cached__near_ridge_kernel(
    x: jax.Array,
    k_cache: jax.Array,
    v_cache: jax.Array,
    wq: jax.Array,
    wo: jax.Array,
):
    nb, sq, d = x.shape
    _, nh, sk, dh = k_cache.shape
    rep = _HQ // nh
    gw = rep * dh
    assert nb & (nb - 1) == 0 and nb > max(_WQ_AT, _WO_AT, _X_HEAD) and nh >= 2
    assert dh % _LANES == 0 and d % 32 == 0
    assert sk % (_NP * _LANES) == 0 and sk % (16 * _NP * _HI_FRAC) == 0
    kern = functools.partial(
        _kernel, nb=nb, nh=nh, rep=rep, sq=sq, sk=sk, dh=dh,
        qscale=(dh ** -0.5) * math.log2(math.e))
    bf16 = jnp.bfloat16
    return pl.pallas_call(
        kern,
        in_specs=[pl.BlockSpec(memory_space=pl.ANY)] * 5,
        out_specs=pl.BlockSpec(memory_space=pl.ANY),
        out_shape=jax.ShapeDtypeStruct((nb, sq, d), x.dtype),
        scratch_shapes=[
            pltpu.VMEM((nb, sq, d), bf16),
            pltpu.VMEM((nh, d, gw), bf16),
            pltpu.VMEM((nh, d, gw), bf16),
            pltpu.VMEM((_NSLOT, sk, dh), bf16),
            pltpu.VMEM((_NSLOT, sk, dh), bf16),
            pltpu.VMEM((nb, rep * sq, dh), bf16),
            pltpu.VMEM((sq, gw), bf16),
            pltpu.VMEM((nb, sq, d), jnp.float32),
            pltpu.VMEM((nb, sq, d), bf16),
            pltpu.SemaphoreType.DMA((2,)),
            pltpu.SemaphoreType.DMA((2 * nh,)),
            pltpu.SemaphoreType.DMA((2 * nh,)),
            pltpu.SemaphoreType.DMA((2 * _NSLOT,)),
            pltpu.SemaphoreType.DMA((2 * _NSLOT,)),
            pltpu.SemaphoreType.DMA((2,)),
            pltpu.SemaphoreType.REGULAR,
        ],
        compiler_params=pltpu.CompilerParams(
            vmem_limit_bytes=64 * 1024 * 1024,
            disable_bounds_checks=True,
        ),
    )(x, k_cache, v_cache, wq, wo.T)
```

```python
import functools
import math

import jax
import jax.numpy as jnp
from jax import lax
import jax.experimental.pallas as pl
import jax.experimental.pallas.tpu as pltpu

_HQ = 16
_NSLOT = 4
_WQ_AT = 1
_WO_AT = 5
_NP = 16
_HI_FRAC = 8
_X_HEAD = 3
_W_PIECE = 32
_LANES = 128
_NT = (((1,), (1,)), ((), ()))


class _Copy:
    def __init__(self, src, dst, sems, first_sem, hi=None):
        self._args = (src, dst, sems, first_sem)
        n = src.shape[0]
        self._hi = n // 2 if hi is None else hi
        self._lo = n - self._hi

    def _part(self, start, size, sem):
        src, dst, sems, first_sem = self._args
        return pltpu.make_async_copy(src.at[pl.ds(start, size)],
                                     dst.at[pl.ds(start, size)],
                                     sems.at[first_sem + sem])

    def start_lo(self, priority=1):
        self._part(0, self._lo, 0).start(priority=priority)

    def start_hi(self):
        self._part(self._lo, self._hi, 1).start(priority=0)

    def start_piece(self, j, count=_NP):
        size = self._hi // count
        start = self._lo + j * size
        if not isinstance(start, int):
            start = pl.multiple_of(start, 16)
        self._part(start, size, 1).start(priority=0)

    def start(self, lo_priority):
        self.start_hi()
        self.start_lo(lo_priority)

    def wait(self):
        self._part(0, self._lo, 0).wait()
        self._part(self._lo, self._hi, 1).wait()


def _kernel(x_hbm, k_hbm, v_hbm, wq_hbm, wot_hbm, o_hbm,
            x_v, wq_v, wot_v, kbuf, vbuf, q_all, o_scr, acc, out_v,
            sem_x, sem_wq, sem_wo, sem_k, sem_v, sem_o, sem_fence,
            *, nb, nh, rep, sq, sk, dh, qscale):
    nsteps = nb * nh
    gw = rep * dh
    ck = sk // _NP
    log_nb = nb.bit_length() - 1
    f32, bf16 = jnp.float32, jnp.bfloat16

    def bh(n):
        if isinstance(n, int):
            return n % nb, n // nb
        return n & (nb - 1), lax.shift_right_logical(n, log_nb)

    def k_copy(n):
        b, h = bh(n)
        slot = n & (_NSLOT - 1)
        return _Copy(k_hbm.at[b, h], kbuf.at[slot], sem_k, 2 * slot, sk // _HI_FRAC)

    def v_copy(n):
        b, h = bh(n)
        slot = n & (_NSLOT - 1)
        return _Copy(v_hbm.at[b, h], vbuf.at[slot], sem_v, 2 * slot, sk // _HI_FRAC)

    def w_slice(w_hbm, h):
        return w_hbm.at[:, pl.ds(pl.multiple_of(h * gw, gw), gw)]

    def wq_copy(h):
        return _Copy(w_slice(wq_hbm, h), wq_v.at[h], sem_wq, 2 * h, _W_PIECE * nb)

    def wo_copy(h):
        return _Copy(w_slice(wot_hbm, h), wot_v.at[h], sem_wo, 2 * h, _W_PIECE * nb)

    x_head_copy = pltpu.make_async_copy(
        x_hbm.at[pl.ds(0, _X_HEAD)], x_v.at[pl.ds(0, _X_HEAD)], sem_x.at[0])
    x_tail_copy = pltpu.make_async_copy(
        x_hbm.at[pl.ds(_X_HEAD, nb - _X_HEAD)], x_v.at[pl.ds(_X_HEAD, nb - _X_HEAD)],
        sem_x.at[1])
    out_head_copy = pltpu.make_async_copy(
        out_v.at[pl.ds(0, nb - 1)], o_hbm.at[pl.ds(0, nb - 1)], sem_o.at[0])
    out_tail_copy = pltpu.make_async_copy(
        out_v.at[pl.ds(nb - 1, 1)], o_hbm.at[pl.ds(nb - 1, 1)], sem_o.at[1])

    def q_proj(b, h):
        q = jnp.dot(x_v[b], wq_v[h], preferred_element_type=f32) * qscale
        q = q.astype(bf16)
        for r in range(rep):
            q_all[b, r * sq:(r + 1) * sq, :] = q[:, r * dh:(r + 1) * dh]

    def o_proj(n):
        b, h = bh(n)
        y = lax.dot_general(o_scr[...], wot_v[h], _NT, preferred_element_type=f32)
        acc[b] = y + jnp.where(h > 0, acc[b], 0.0)

    def scores(b, slot, issue):
        q = q_all[b]
        parts = []
        for c in range(_NP):
            parts.append(lax.dot_general(q, kbuf[slot, c * ck:(c + 1) * ck, :], _NT,
                                         preferred_element_type=f32))
            issue(c)
        return jnp.concatenate(parts, axis=1)

    def weighted_values(p, slot, issue):
        o = None
        for c in range(_NP):
            oc = jnp.dot(p[:, c * ck:(c + 1) * ck], vbuf[slot, c * ck:(c + 1) * ck, :],
                         preferred_element_type=f32)
            o = oc if o is None else o + oc
            issue(c)
        return o

    wq_copy(0).start(0)
    x_head_copy.start()
    x_tail_copy.start()
    k_copy(0).start(0)
    wo_copy(0).start(0)
    wq_copy(1).start(0)
    v_copy(0).start(1)
    k_copy(1).start_lo()
    v_copy(1).start_lo()
    k_copy(2).start_lo()
    v_copy(2).start_lo()
    o_scr[...] = jnp.zeros(o_scr.shape, o_scr.dtype)
    wq_copy(0).wait()
    x_head_copy.wait()
    for b in range(_X_HEAD):
        q_proj(b, 0)
    x_tail_copy.wait()
    for b in range(_X_HEAD, nb):
        q_proj(b, 0)
    wo_copy(0).wait()

    def main_body(n, carry):
        b, h = bh(n)
        slot = n & (_NSLOT - 1)

        @pl.when(jnp.logical_and(b == 1, h > 0))
        def _():
            wo_copy(h).wait()

        k_copy(n).wait()

        @pl.when(jnp.logical_and(b == _WQ_AT, h + 2 < nh))
        def _():
            wq_copy(h + 2).start_lo()

        @pl.when(b == _WO_AT)
        def _():
            wo_copy(h + 1).start_lo()

        s = scores(b, slot, k_copy(n + 1).start_piece)
        o_proj(jnp.maximum(n - 1, 0))
        wo_copy(h + 1).start_piece(b, nb)
        m = jnp.max(s, axis=-1, keepdims=True)

        k_copy(n + 3).start_lo()

        @pl.when(b == 0)
        def _():
            wq_copy(h + 1).wait()

        v_copy(n).wait()

        q_proj(b, h + 1)

        @pl.when(h + 2 < nh)
        def _():
            wq_copy(h + 2).start_piece(b, nb)

        p = jnp.exp2(s - m)
        l = jnp.sum(p, axis=-1, keepdims=True)
        o = weighted_values(p.astype(bf16), slot, v_copy(n + 1).start_piece)
        o = (o / l).astype(bf16)
        for r in range(rep):
            o_scr[:, r * dh:(r + 1) * dh] = o[r * sq:(r + 1) * sq, :]
        v_copy(n + 3).start_lo()
        return carry

    def last_body(n, carry):
        b = n & (nb - 1)
        h = nh - 1
        slot = n & (_NSLOT - 1)

        @pl.when(b == 0)
        def _():
            wo_copy(h).wait()

        k_copy(n).wait()

        def issue_k(c):
            @pl.when(b < nb - 1)
            def _():
                k_copy(n + 1).start_piece(c)

        s = scores(b, slot, issue_k)
        m = jnp.max(s, axis=-1, keepdims=True)

        @pl.when(b < nb - 3)
        def _():
            k_copy(n + 3).start_lo()

        @pl.when(b < nb - 1)
        def _():
            v_copy(n).wait()
            v_copy(n + 1).start_hi()

        @pl.when(b == nb - 1)
        def _():
            v_copy(n).wait()
            out_head_copy.start()

        pl.semaphore_signal(sem_fence, 1)
        pl.semaphore_wait(sem_fence, 1)

        p = jnp.exp2(s - m)
        l = jnp.sum(p, axis=-1, keepdims=True)
        p = p.astype(bf16)
        y = acc[b]
        chunks = []
        for c in range(dh // _LANES):
            oc = jnp.dot(p, vbuf[slot, :, c * _LANES:(c + 1) * _LANES],
                         preferred_element_type=f32)
            chunks.append((oc / l).astype(bf16))
        for c, oc in enumerate(chunks):
            for r in range(rep):
                col = r * dh + c * _LANES
                y = y + lax.dot_general(oc[r * sq:(r + 1) * sq, :],
                                        wot_v[h, :, col:col + _LANES], _NT,
                                        preferred_element_type=f32)
        out_v[b] = y.astype(out_v.dtype)

        @pl.when(b < nb - 3)
        def _():
            v_copy(n + 3).start_lo()

        return carry

    lax.fori_loop(0, nsteps - nb, main_body, 0)
    o_proj(nsteps - nb - 1)
    lax.fori_loop(nsteps - nb, nsteps, last_body, 0)

    out_tail_copy.start()
    out_head_copy.wait()
    out_tail_copy.wait()


@jax.jit
def pallas_standalone__gqa_block_cached__near_ridge_kernel(
    x: jax.Array,
    k_cache: jax.Array,
    v_cache: jax.Array,
    wq: jax.Array,
    wo: jax.Array,
):
    nb, sq, d = x.shape
    _, nh, sk, dh = k_cache.shape
    rep = _HQ // nh
    gw = rep * dh
    assert nb & (nb - 1) == 0 and nb > max(_WQ_AT, _WO_AT, _X_HEAD) and nh >= 2
    assert dh % _LANES == 0 and d % 16 == 0 and d > _W_PIECE * nb and _W_PIECE % 16 == 0
    assert sk % (_NP * _LANES) == 0 and sk % (16 * _NP * _HI_FRAC) == 0
    kern = functools.partial(
        _kernel, nb=nb, nh=nh, rep=rep, sq=sq, sk=sk, dh=dh,
        qscale=(dh ** -0.5) * math.log2(math.e))
    bf16 = jnp.bfloat16
    return pl.pallas_call(
        kern,
        in_specs=[pl.BlockSpec(memory_space=pl.ANY)] * 5,
        out_specs=pl.BlockSpec(memory_space=pl.ANY),
        out_shape=jax.ShapeDtypeStruct((nb, sq, d), x.dtype),
        scratch_shapes=[
            pltpu.VMEM((nb, sq, d), bf16),
            pltpu.VMEM((nh, d, gw), bf16),
            pltpu.VMEM((nh, d, gw), bf16),
            pltpu.VMEM((_NSLOT, sk, dh), bf16),
            pltpu.VMEM((_NSLOT, sk, dh), bf16),
            pltpu.VMEM((nb, rep * sq, dh), bf16),
            pltpu.VMEM((sq, gw), bf16),
            pltpu.VMEM((nb, sq, d), jnp.float32),
            pltpu.VMEM((nb, sq, d), bf16),
            pltpu.SemaphoreType.DMA((2,)),
            pltpu.SemaphoreType.DMA((2 * nh,)),
            pltpu.SemaphoreType.DMA((2 * nh,)),
            pltpu.SemaphoreType.DMA((2 * _NSLOT,)),
            pltpu.SemaphoreType.DMA((2 * _NSLOT,)),
            pltpu.SemaphoreType.DMA((2,)),
            pltpu.SemaphoreType.REGULAR,
        ],
        compiler_params=pltpu.CompilerParams(
            vmem_limit_bytes=64 * 1024 * 1024,
            disable_bounds_checks=True,
        ),
    )(x, k_cache, v_cache, wq, wo.T)
```
